```python
import os as _os
_os.environ.setdefault("JAX_PLATFORMS", "cpu")
import jax
import jax.numpy as jnp

def _softmax(x, axis=-1):
    return jax.nn.softmax(x, axis=axis)
def _gelu(x):
    return jax.nn.gelu(x, approximate=True)
def _silu(x):
    return jax.nn.silu(x)
def _sigmoid(x):
    return jax.nn.sigmoid(x)
def _layernorm(x, axis=-1, eps=1e-5):
    m = jnp.mean(x, axis=axis, keepdims=True)
    v = jnp.var(x, axis=axis, keepdims=True)
    return (x - m) / jnp.sqrt(v + eps)
def _scatter_add(tgt, idx, src, axis=0):
    return tgt.at[idx].add(src)
def _segment_sum(src, seg, n):
    return jax.ops.segment_sum(src, seg, n)
class _Rng:
    def __init__(self, key):
        self._k = key
    def _next(self):
        self._k, sub = jax.random.split(self._k)
        return sub
    def normal(self, shape):
        return jax.random.normal(self._next(), shape, dtype=jnp.bfloat16)
    def randint(self, lo, hi, shape):
        return jax.random.randint(self._next(), shape, lo, hi, dtype=jnp.int32)
    def uniform(self, shape, lo=0.0, hi=1.0):
        return jax.random.uniform(self._next(), shape, jnp.bfloat16, lo, hi)
    def permutation(self, n):
        return jax.random.permutation(self._next(), n)


kernel_name = 'concat_heads__gqa_block_cached__mha_block_cached__near_ridge'

def setup_inputs():
    _rng = _Rng(jax.random.key(int.from_bytes(__import__("os").urandom(4), "little")))
    _w = (lambda a: (lambda t: t.astype(jnp.bfloat16) if jnp.issubdtype(t.dtype, jnp.floating) else t)(jnp.asarray(a)))
    def _A_setup():
        B, Sq, D = 8, 96, 640
        Hq, Hkv, Sk, Dh = 32, 32, 512, 128
        assert Hq % Hkv == 0, (Hq, Hkv)
        return {
            "x": _w((lambda *s: _rng.normal(s) * 0.8)(B, Sq, D)),
            "k_cache": _w((lambda *s: _rng.normal(s) * 0.8)(B, Hkv, Sk, Dh)),
            "v_cache": _w((lambda *s: _rng.normal(s) * 0.05)(B, Hkv, Sk, Dh)),
            "wq": _w((lambda *s: _rng.normal(s) * 0.8)(D, Hq * Dh) * (D ** -0.5)),
            "wo": _w((lambda *s: _rng.normal(s) * 0.05)(Hq * Dh, D) * ((Hq * Dh) ** -0.5)),
        }
    _A_in = _A_setup()

    def _B_setup():
        B, Sq, D = 8, 96, 640
        H, Sk, Dh = 32, 512, 128
        return {
            "x": _w((lambda *s: _rng.normal(s) * 0.8)(B, Sq, D)),
            "k_cache": _w((lambda *s: _rng.normal(s) * 0.8)(B, H, Sk, Dh)),
            "v_cache": _w((lambda *s: _rng.normal(s) * 0.05)(B, H, Sk, Dh)),
            "wq": _w((lambda *s: _rng.normal(s) * 0.8)(D, H * Dh) * (D ** -0.5)),
            "wo": _w((lambda *s: _rng.normal(s) * 0.05)(H * Dh, D) * ((H * Dh) ** -0.5)),
        }
    _B_in = _B_setup()

    return {
        "A_x": _A_in["x"],
        "A_k_cache": _A_in["k_cache"],
        "A_v_cache": _A_in["v_cache"],
        "A_wq": _A_in["wq"],
        "A_wo": _A_in["wo"],
        "B_x": _B_in["x"],
        "B_k_cache": _B_in["k_cache"],
        "B_v_cache": _B_in["v_cache"],
        "B_wq": _B_in["wq"],
        "B_wo": _B_in["wo"],
    }

def reference(A_x, A_k_cache, A_v_cache, A_wq, A_wo, B_x, B_k_cache, B_v_cache, B_wq, B_wo):
    def _A_ref(x, k_cache, v_cache, wq, wo):
        B, Sq, D = x.shape
        Hq, Dh = 32, 128
        Hkv = k_cache.shape[1]
        rep = Hq // Hkv
        q = (lambda x, *d: x.transpose(*d))((x @ wq).reshape(B, Sq, Hq, Dh), 0, 2, 1, 3)
        k = jnp.repeat(k_cache, rep, axis=1)
        v = jnp.repeat(v_cache, rep, axis=1)
        scores = jnp.einsum("bhqd,bhkd->bhqk", q, k) * (Dh ** -0.5)
        p = _softmax(scores, axis=-1)
        o = jnp.einsum("bhqk,bhkd->bhqd", p, v)
        return (lambda x, *d: x.transpose(*d))(o, 0, 2, 1, 3).reshape(B, Sq, Hq * Dh) @ wo

    def _B_ref(x, k_cache, v_cache, wq, wo):
        B, Sq, D = x.shape
        H, Dh = 32, 128
        q = (lambda x, *d: x.transpose(*d))((x @ wq).reshape(B, Sq, H, Dh), 0, 2, 1, 3)
        scores = jnp.einsum("bhqd,bhkd->bhqk", q, k_cache) * (Dh ** -0.5)
        p = _softmax(scores, axis=-1)
        o = jnp.einsum("bhqk,bhkd->bhqd", p, v_cache)
        return (lambda x, *d: x.transpose(*d))(o, 0, 2, 1, 3).reshape(B, Sq, H * Dh) @ wo

    a = _A_ref(A_x, A_k_cache, A_v_cache, A_wq, A_wo)
    b = _B_ref(B_x, B_k_cache, B_v_cache, B_wq, B_wo)
    return jnp.concatenate([a, b], axis=-1)
```

```python
import functools
import jax, jax.numpy as jnp
from jax import lax
import jax.experimental.pallas as pl
import jax.experimental.pallas.tpu as pltpu

B, SQ, D, H, SK, DH = 8, 96, 640, 32, 512, 128
M = B * SQ
NT = 2 * H
LOG2E = 1.4426950408889634

def build(NB=6, nsplit=8, prio=True, nodma=False, order='seq', flags=None, mchunk=96):
    NW = NB + 2
    scale = DH ** -0.5 * LOG2E
    def kern(Ax, Ak, Av, Awq, Awo, Bx, Bk, Bv, Bwq, Bwo, out,
             xb, kb, vb, wqb, wob, qb, ob, acc, resb, sem_x, sem_k, sem_v, sem_wq, sem_wo, sem_o):
        bs = B // nsplit
        def start_kv(k, v, h, slot):
            for src, dst, sem in ((k, kb, sem_k), (v, vb, sem_v)):
                for s in range(nsplit):
                    pltpu.make_async_copy(src.at[pl.ds(s*bs, bs), h], dst.at[slot, pl.ds(s*bs, bs)], sem.at[slot]).start(priority=(s % 2) if prio else 0)
        def start_wq(wq, h, slot):
            pltpu.make_async_copy(wq.at[:, pl.ds(pl.multiple_of(h * DH, DH), DH)], wqb.at[slot], sem_wq.at[slot]).start()
        def start_wo(wo, h, slot):
            pltpu.make_async_copy(wo.at[pl.ds(pl.multiple_of(h * DH, DH), DH), :], wob.at[slot], sem_wo.at[slot]).start()
        def wait(buf, sem, slot):
            pltpu.make_async_copy(buf.at[slot], buf.at[slot], sem.at[slot]).wait()

        def qproj(br, wslot, qslot, r0, n):
            q = jnp.dot(xb[br, pl.ds(r0, n), :], wqb[wslot], preferred_element_type=jnp.float32)
            qb[qslot, pl.ds(r0, n), :] = (q * scale).astype(jnp.bfloat16)
        def scores(slot, qslot, b):
            return lax.dot_general(qb[qslot, pl.ds(b*SQ, SQ), :], kb[slot, b], (((1,), (1,)), ((), ())), preferred_element_type=jnp.float32)
        def soft(s):
            m = jnp.max(s, axis=-1, keepdims=True)
            p = jnp.exp2(s - m)
            l = jnp.sum(p, axis=-1, keepdims=True)
            return p.astype(jnp.bfloat16), l
        def pv(p, l, slot, oslot, b):
            o = jnp.dot(p, vb[slot, b], preferred_element_type=jnp.float32)
            ob[oslot, pl.ds(b*SQ, SQ), :] = (o * (1.0 / l)).astype(jnp.bfloat16)
        def oproj(oslot, wslot, r0, n):
            acc[pl.ds(r0, n), :] += jnp.dot(ob[oslot, pl.ds(r0, n), :], wob[wslot], preferred_element_type=jnp.float32)

        pltpu.make_async_copy(Ax, xb.at[0], sem_x.at[0]).start()
        start_wq(Awq, 0, 0)
        for j in range(NB - 1):
            start_kv(Ak, Av, j, j)
            start_wq(Awq, j + 1, j + 1)
            start_wo(Awo, j, j)
        pltpu.make_async_copy(Bx, xb.at[1], sem_x.at[1]).start()
        wait(xb, sem_x, 0)
        wait(wqb, sem_wq, 0)
        qproj(0, 0, 0, 0, M)
        ob[1] = jnp.zeros((M, DH), jnp.bfloat16)
        wob[NW - 1] = jnp.zeros((DH, D), jnp.bfloat16)
        acc[...] = jnp.zeros_like(acc)

        def step(t, c):
            n = t + NB - 1
            if not nodma:
                @pl.when(n < H)
                def _():
                    start_kv(Ak, Av, n, n % NB)
                    start_wo(Awo, n, n % NW)
                @pl.when(jnp.logical_and(n >= H, n < NT))
                def _():
                    start_kv(Bk, Bv, n - H, n % NB)
                    start_wo(Bwo, n - H, n % NW)
                @pl.when(n + 1 < H)
                def _():
                    start_wq(Awq, n + 1, (n + 1) % NW)
                @pl.when(jnp.logical_and(n + 1 >= H, n + 1 < NT))
                def _():
                    start_wq(Bwq, n + 1 - H, (n + 1) % NW)
            @pl.when(t == H - 1)
            def _():
                wait(xb, sem_x, 1)
            @pl.when(t == H + 1)
            def _():
                resb[0] = acc[...].astype(jnp.bfloat16)
                pltpu.make_async_copy(resb.at[0], out.at[:, pl.ds(0, D)], sem_o.at[0]).start()
                acc[...] = jnp.zeros_like(acc)
            slot = t % NB
            def waits():
                @pl.when(t + 1 < NT)
                def _():
                    wait(wqb, sem_wq, (t + 1) % NW)
                @pl.when(t > 0)
                def _():
                    wait(wob, sem_wo, (t - 1) % NW)
                wait(kb, sem_k, slot)
                wait(vb, sem_v, slot)
            if nodma:
                pl.when(t < NB - 1)(waits)
                @pl.when(t == NB - 1)
                def _():
                    wait(wob, sem_wo, (t - 1) % NW)
            else:
                waits()
            br = jnp.minimum((t + 1) // H, 1)
            wq_s = (t + 1) % NW
            wo_s = (t + NW - 1) % NW
            cur = t % 2
            nxt = 1 - cur
            if order == 'seq':
                qproj(br, wq_s, nxt, 0, M)
                for b in range(B):
                    p, l = soft(scores(slot, cur, b))
                    pv(p, l, slot, cur, b)
                oproj(nxt, wo_s, 0, M)
            elif order == 'il':
                nm = M // mchunk
                per = B // nm
                s = scores(slot, cur, 0)
                for b in range(B):
                    s_next = scores(slot, cur, b + 1) if b + 1 < B else None
                    if b % per == 0:
                        qproj(br, wq_s, nxt, (b // per) * mchunk, mchunk)
                    p, l = soft(s)
                    if b % per == per - 1:
                        oproj(nxt, wo_s, (b // per) * mchunk, mchunk)
                    pv(p, l, slot, cur, b)
                    s = s_next
            return c
        lax.fori_loop(0, NT, step, 0)
        if not nodma:
            wait(wob, sem_wo, (NT - 1) % NW)
        oproj((NT - 1) % 2, (NT - 1) % NW, 0, M)
        resb[1] = acc[...].astype(jnp.bfloat16)
        cp = pltpu.make_async_copy(resb.at[1], out.at[:, pl.ds(D, D)], sem_o.at[1])
        cp.start()
        pltpu.make_async_copy(resb.at[0], out.at[:, pl.ds(0, D)], sem_o.at[0]).wait()
        cp.wait()

    bf = jnp.bfloat16
    def fn(Ax, Ak, Av, Awq, Awo, Bx, Bk, Bv, Bwq, Bwo):
        r = pl.pallas_call(kern,
            in_specs=[pl.BlockSpec(memory_space=pl.ANY)] * 10,
            out_specs=pl.BlockSpec(memory_space=pl.ANY),
            out_shape=jax.ShapeDtypeStruct((M, 2 * D), bf),
            scratch_shapes=[pltpu.VMEM((2, M, D), bf), pltpu.VMEM((NB, B, SK, DH), bf), pltpu.VMEM((NB, B, SK, DH), bf),
                pltpu.VMEM((NW, D, DH), bf), pltpu.VMEM((NW, DH, D), bf), pltpu.VMEM((2, M, DH), bf), pltpu.VMEM((2, M, DH), bf),
                pltpu.VMEM((M, D), jnp.float32), pltpu.VMEM((2, M, D), bf),
                pltpu.SemaphoreType.DMA((2,)), pltpu.SemaphoreType.DMA((NB,)), pltpu.SemaphoreType.DMA((NB,)),
                pltpu.SemaphoreType.DMA((NW,)), pltpu.SemaphoreType.DMA((NW,)), pltpu.SemaphoreType.DMA((2,))],
            compiler_params=pltpu.CompilerParams(vmem_limit_bytes=100 * 2**20, flags=flags),
        )(Ax.reshape(M, D), Ak, Av, Awq, Awo, Bx.reshape(M, D), Bk, Bv, Bwq, Bwo)
        return r.reshape(B, SQ, 2 * D)
    return fn


@jax.jit
def pallas_concat_heads__gqa_block_cached__mha_block_cached__near_ridge_kernel(A_x, A_k_cache, A_v_cache, A_wq, A_wo, B_x, B_k_cache, B_v_cache, B_wq, B_wo):
    return build(order='il', NB=4, nsplit=1, prio=False)(A_x, A_k_cache, A_v_cache, A_wq, A_wo, B_x, B_k_cache, B_v_cache, B_wq, B_wo)
```

```python
import jax
import jax.experimental.pallas as pl
import jax.experimental.pallas.tpu as pltpu
import jax.numpy as jnp
from jax import lax

B, SQ, D, H, SK, DH = 8, 96, 640, 32, 512, 128
M = B * SQ
STEPS = 2 * H
LOG2E = 1.4426950408889634

KV_AHEAD = 2
KV_SLOTS = KV_AHEAD + 1
KV_ROWS = 128
KV_PARTS = SK // KV_ROWS
Q_AHEAD = 8
Q_SLOTS = Q_AHEAD + 1
WQ_GROUP = 16
WQ_AHEAD = WQ_GROUP + Q_AHEAD
WO_GROUP = 8
WO_SLOTS = 3
W_PIECES = 5
COL_TILES = D // 128
PIECE_TILES = 16
X_PIECES = M // 8 * COL_TILES // PIECE_TILES
HEAD_TILES = DH // 8 * COL_TILES
BATCH_TILES = SQ // 8 * COL_TILES

SEM_X = 0
SEM_OUT = SEM_X + 2
SEM_K = SEM_OUT + 2
SEM_V = SEM_K + KV_SLOTS
SEM_WO = SEM_V + KV_SLOTS
SEM_WQ = SEM_WO + WO_SLOTS
NUM_SEMS = SEM_WQ + STEPS // WQ_GROUP


def _as_tiles(a):
    r, c = a.shape
    a = a.reshape(r // 8, 8, c // 128, 128).transpose(0, 2, 1, 3)
    return a.reshape(r // 8 * (c // 128), 8, 128)


def _from_tiles(v):
    n = v.shape[0] // COL_TILES
    v = v.reshape(n, COL_TILES, 8, 128)
    return jnp.concatenate([v[:, c].reshape(n * 8, 128) for c in range(COL_TILES)], axis=1)


def _kernel(a_x, a_k, a_v, a_wq, a_wo, b_x, b_k, b_v, b_wq, b_wo, out,
            x_buf, k_buf, v_buf, wq_buf, wo_buf, q_buf, acc, res, sem):
    copy = pltpu.make_async_copy

    def x_copy(br, piece):
        tiles = pl.ds(piece * PIECE_TILES, PIECE_TILES)
        return copy((a_x, b_x)[br].at[tiles], x_buf.at[br, tiles], sem.at[SEM_X + br])

    def wq_copy(br, m, i):
        group = m // WQ_GROUP
        width = WQ_GROUP * DH
        cols = pl.ds(pl.multiple_of(group * width, width), width)
        rows = pl.ds(pl.multiple_of((i * WQ_GROUP + m % WQ_GROUP) * 8, 8), 8)
        slot = br * (H // WQ_GROUP) + group
        return copy((a_wq, b_wq)[br].at[rows, cols], wq_buf.at[slot, rows], sem.at[SEM_WQ + slot])

    def wo_copy(br, m, i):
        group = m // WO_GROUP
        tile = (i * WO_GROUP + m % WO_GROUP) * PIECE_TILES
        slot = (br * (H // WO_GROUP) + group) % WO_SLOTS
        return copy((a_wo, b_wo)[br].at[pl.ds(group * (WO_GROUP * HEAD_TILES) + tile, PIECE_TILES)],
                    wo_buf.at[slot, pl.ds(tile, PIECE_TILES)], sem.at[SEM_WO + slot])

    def kv_copy(br, h, slot, is_v, part, b):
        src, dst, base = (((a_k, b_k)[br], k_buf, SEM_K), ((a_v, b_v)[br], v_buf, SEM_V))[is_v]
        rows = pl.ds(pl.multiple_of(part * KV_ROWS, KV_ROWS), KV_ROWS)
        return copy(src.at[b, h, rows], dst.at[slot, b, rows], sem.at[base + slot])

    def out_copy(br, row, n):
        rows = pl.ds(row, n)
        return copy(res.at[br, rows], out.at[rows, pl.ds(br * D, D)], sem.at[SEM_OUT + br])

    def wait_all(buf, base, slot):
        copy(buf.at[slot], buf.at[slot], sem.at[base + slot]).wait()

    def starter(make, *args):
        return lambda priority: make(*args).start(priority=priority)

    def step_starter(make, n, lo, hi):
        def start(priority):
            for br in range(2):
                if lo >= br * H and hi <= (br + 1) * H:
                    make(br, n - br * H).start(priority=priority)
                elif lo < (br + 1) * H and hi > br * H:
                    @pl.when(n // H == br)
                    def _():
                        make(br, n - br * H).start(priority=priority)
        return [start] if lo < STEPS else []

    def fetch_list(n, lo, hi):
        starts = []
        for is_v, pieces in enumerate((range(0, 2), range(2, W_PIECES))):
            for make, ahead in ((wq_copy, WQ_AHEAD), (wo_copy, WO_GROUP)):
                for i in pieces:
                    starts += step_starter(lambda br, m, make=make, i=i: make(br, m, i),
                                           n + ahead, lo + ahead, hi + ahead)
            for part in range(KV_PARTS):
                for b in range(B):
                    starts += step_starter(
                        lambda br, h, c=(is_v, part, b): kv_copy(br, h, n % KV_SLOTS, *c), n, lo, hi)
        return starts

    def issue(starts, chunk=0, chunks=1, first=0):
        for i in range(len(starts) * chunk // chunks, len(starts) * (chunk + 1) // chunks):
            starts[i]((first + i) % 2)

    def batch_rows(b):
        return pl.ds(b * SQ, SQ)

    def q_proj(t, b):
        x = _from_tiles(x_buf[t // H, pl.ds(b * BATCH_TILES, BATCH_TILES)])
        w = wq_buf[t // WQ_GROUP, :, pl.ds(pl.multiple_of((t % WQ_GROUP) * DH, DH), DH)]
        q = jnp.dot(x, w, preferred_element_type=jnp.float32)
        return (q * (DH ** -0.5 * LOG2E)).astype(jnp.bfloat16)

    def scores(t, b):
        return lax.dot_general(q_buf[t % Q_SLOTS, batch_rows(b), :], k_buf[t % KV_SLOTS, b],
                               (((1,), (1,)), ((), ())), preferred_element_type=jnp.float32)

    def softmax_terms(s):
        p = jnp.exp2(s - jnp.max(s, axis=-1, keepdims=True))
        return p.astype(jnp.bfloat16), jnp.sum(p, axis=-1, keepdims=True)

    def attend(t, b, p, total):
        o = jnp.dot(p, v_buf[t % KV_SLOTS, b], preferred_element_type=jnp.float32)
        return (o * (1.0 / total)).astype(jnp.bfloat16)

    def out_proj(t, o):
        tiles = pl.ds((t % WO_GROUP) * HEAD_TILES, HEAD_TILES)
        w = _from_tiles(wo_buf[(t // WO_GROUP) % WO_SLOTS, tiles])
        return jnp.dot(o, w, preferred_element_type=jnp.float32)

    issue([starter(x_copy, 0, p) for p0 in range(5) for p in range(p0, X_PIECES, 5)])
    for make, ahead in ((wq_copy, WQ_AHEAD), (wo_copy, WO_GROUP)):
        def fetch_weights(j, carry, make=make):
            issue([starter(make, 0, 2 * j + u, i) for u in range(2) for i in range(W_PIECES)])
            return carry
        lax.fori_loop(0, (ahead + KV_AHEAD) // 2, fetch_weights, 0)
    x_per_iter = X_PIECES // Q_AHEAD
    issue([starter(x_copy, 1, p) for p in range(x_per_iter * Q_AHEAD, X_PIECES)])
    wait_all(x_buf, SEM_X, 0)
    wait_all(wq_buf, SEM_WQ, 0)

    def warm_up(j, carry):
        n = j // KV_PARTS
        starts = [starter(kv_copy, 0, n, n, is_v, j % KV_PARTS, b) for is_v in range(2) for b in range(B)]
        starts += [starter(x_copy, 1, i * Q_AHEAD + j) for i in range(x_per_iter)]
        for b in range(B):
            issue(starts, b, B)
            q_buf[j, batch_rows(b), :] = q_proj(j, b)
        n_rows = M // Q_AHEAD
        for br in range(2):
            acc[br, pl.ds(pl.multiple_of(j * n_rows, n_rows), n_rows), :] = jnp.zeros((n_rows, D), jnp.float32)
        return carry

    lax.fori_loop(0, Q_AHEAD, warm_up, 0)

    def step(t, lo, hi):
        last = lo == STEPS - 1
        with_q = lo + Q_AHEAD < STEPS
        lag = 1 if with_q else 2
        starts = fetch_list(t + KV_AHEAD, lo + KV_AHEAD, hi + KV_AHEAD)

        def at_step(t0, f):
            if lo <= t0 < hi:
                pl.when(t == t0)(f)

        def finish_a():
            res[0] = acc[0].astype(jnp.bfloat16)

        def write_a():
            issue([starter(out_copy, 0, row, 2 * SQ) for row in range(0, M, 2 * SQ)])

        def accumulate(b, o):
            if not last:
                acc[t // H, batch_rows(b), :] += out_proj(t, o)
                return
            res[1, batch_rows(b), :] = (acc[1, batch_rows(b), :] + out_proj(t, o)).astype(jnp.bfloat16)
            issue([starter(out_copy, 1, row, 32) for row in range(b * SQ, (b + 1) * SQ, 32)], first=b)

        at_step(H - Q_AHEAD, lambda: wait_all(x_buf, SEM_X, 1))
        at_step(H, finish_a)
        if with_q:
            pl.when((t + Q_AHEAD) % WQ_GROUP == 0)(
                lambda: wait_all(wq_buf, SEM_WQ, (t + Q_AHEAD) // WQ_GROUP))
        if not last:
            pl.when(t % WO_GROUP == 0)(lambda: wait_all(wo_buf, SEM_WO, (t // WO_GROUP) % WO_SLOTS))
        wait_all(k_buf, SEM_K, t % KV_SLOTS)

        s = {b: scores(t, b) for b in range(lag)}
        o = {}
        q = None
        for b in range(B):
            issue(starts, 2 * b, 2 * B)
            if b == B - 1:
                at_step(STEPS - 2, write_a)
            if b + lag < B:
                s[b + lag] = scores(t, b + lag)
            if q is not None:
                q_buf[(t + Q_AHEAD) % Q_SLOTS, batch_rows(b - 1), :] = q
            p, total = softmax_terms(s.pop(b))
            issue(starts, 2 * b + 1, 2 * B)
            if b >= lag:
                accumulate(b - lag, o.pop(b - lag))
            if b == 0:
                wait_all(v_buf, SEM_V, t % KV_SLOTS)
            o[b] = attend(t, b, p, total)
            if with_q:
                q = q_proj(t + Q_AHEAD, b)
        for b in range(B - lag, B):
            accumulate(b, o.pop(b))
        if with_q:
            q_buf[(t + Q_AHEAD) % Q_SLOTS, batch_rows(B - 1), :] = q

    for lo, hi in ((0, STEPS - Q_AHEAD), (STEPS - Q_AHEAD, STEPS - 1)):
        def body(t, carry, lo=lo, hi=hi):
            step(t, lo, hi)
            return carry
        lax.fori_loop(lo, hi, body, 0)
    step(STEPS - 1, STEPS - 1, STEPS)
    for br in range(2):
        out_copy(br, 0, M).wait()


@jax.jit
def pallas_concat_heads__gqa_block_cached__mha_block_cached__near_ridge_kernel(
    A_x: jax.Array,
    A_k_cache: jax.Array,
    A_v_cache: jax.Array,
    A_wq: jax.Array,
    A_wo: jax.Array,
    B_x: jax.Array,
    B_k_cache: jax.Array,
    B_v_cache: jax.Array,
    B_wq: jax.Array,
    B_wo: jax.Array,
):
    assert A_x.shape == B_x.shape == (B, SQ, D)
    assert A_k_cache.shape == A_v_cache.shape == B_k_cache.shape == B_v_cache.shape == (B, H, SK, DH)
    bf16 = jnp.bfloat16
    out = pl.pallas_call(
        _kernel,
        in_specs=[pl.BlockSpec(memory_space=pl.ANY)] * 10,
        out_specs=pl.BlockSpec(memory_space=pl.ANY),
        out_shape=jax.ShapeDtypeStruct((M, 2 * D), bf16),
        scratch_shapes=[
            pltpu.VMEM((2, B * BATCH_TILES, 8, 128), bf16),
            pltpu.VMEM((KV_SLOTS, B, SK, DH), bf16),
            pltpu.VMEM((KV_SLOTS, B, SK, DH), bf16),
            pltpu.VMEM((STEPS // WQ_GROUP, D, WQ_GROUP * DH), bf16),
            pltpu.VMEM((WO_SLOTS, WO_GROUP * HEAD_TILES, 8, 128), bf16),
            pltpu.VMEM((Q_SLOTS, M, DH), bf16),
            pltpu.VMEM((2, M, D), jnp.float32),
            pltpu.VMEM((2, M, D), bf16),
            pltpu.SemaphoreType.DMA((NUM_SEMS,)),
        ],
        compiler_params=pltpu.CompilerParams(
            vmem_limit_bytes=64 * 2**20, disable_bounds_checks=True, disable_semaphore_checks=True),
    )(
        _as_tiles(A_x.reshape(M, D)), A_k_cache, A_v_cache, A_wq, _as_tiles(A_wo),
        _as_tiles(B_x.reshape(M, D)), B_k_cache, B_v_cache, B_wq, _as_tiles(B_wo),
    )
    return out.reshape(B, SQ, 2 * D)
```
